```python
import os as _os
_os.environ.setdefault("JAX_PLATFORMS", "cpu")
import jax
import jax.numpy as jnp

def _softmax(x, axis=-1):
    return jax.nn.softmax(x, axis=axis)
def _gelu(x):
    return jax.nn.gelu(x, approximate=True)
def _silu(x):
    return jax.nn.silu(x)
def _sigmoid(x):
    return jax.nn.sigmoid(x)
def _layernorm(x, axis=-1, eps=1e-5):
    m = jnp.mean(x, axis=axis, keepdims=True)
    v = jnp.var(x, axis=axis, keepdims=True)
    return (x - m) / jnp.sqrt(v + eps)
def _scatter_add(tgt, idx, src, axis=0):
    return tgt.at[idx].add(src)
def _segment_sum(src, seg, n):
    return jax.ops.segment_sum(src, seg, n)
class _Rng:
    def __init__(self, key):
        self._k = key
    def _next(self):
        self._k, sub = jax.random.split(self._k)
        return sub
    def normal(self, shape):
        return jax.random.normal(self._next(), shape, dtype=jnp.bfloat16)
    def randint(self, lo, hi, shape):
        return jax.random.randint(self._next(), shape, lo, hi, dtype=jnp.int32)
    def uniform(self, shape, lo=0.0, hi=1.0):
        return jax.random.uniform(self._next(), shape, jnp.bfloat16, lo, hi)
    def permutation(self, n):
        return jax.random.permutation(self._next(), n)


kernel_name = 'parallel_sum__ssm_conv_s5__geglu_ffn__prompt'

def setup_inputs():
    _rng = _Rng(jax.random.key(int.from_bytes(__import__("os").urandom(4), "little")))
    _w = (lambda a: (lambda t: t.astype(jnp.bfloat16) if jnp.issubdtype(t.dtype, jnp.floating) else t)(jnp.asarray(a)))
    def _A_setup():
        B, S, D = 1, 2048, 512
        P = D
        Lambda_re = -0.5 * jnp.exp((lambda *s: _rng.normal(s) * 0.8)(P))
        Lambda_im = (lambda *s: _rng.normal(s) * 0.8)(P) * 1.0
        B_re = (lambda *s: _rng.normal(s) * 0.8)(P, D) * (D ** -0.5)
        B_im = (lambda *s: _rng.normal(s) * 0.8)(P, D) * (D ** -0.5)
        C_re = (lambda *s: _rng.normal(s) * 0.8)(D, P) * (P ** -0.5)
        C_im = (lambda *s: _rng.normal(s) * 0.8)(D, P) * (P ** -0.5)
        log_dt = (lambda *s: _rng.normal(s) * 0.8)(P) * 0.3 - 2.0
        Dskip = (lambda *s: _rng.normal(s) * 0.8)(D)
        return {
            "x": _w((lambda *s: _rng.normal(s) * 0.05)(B, S, D)),
            "Lambda_re": _w(Lambda_re),
            "Lambda_im": _w(Lambda_im),
            "B_re": _w(B_re),
            "B_im": _w(B_im),
            "C_re": _w(C_re),
            "C_im": _w(C_im),
            "log_dt": _w(log_dt),
            "Dskip": _w(Dskip),
        }
    _A_in = _A_setup()

    def _B_setup():
        B, S, D, F = 1, 2048, 512, 1376
        return {
            "x": _w((lambda *s: _rng.normal(s) * 0.05)(B, S, D)),
            "w_gate": _w((lambda *s: _rng.normal(s) * 0.05)(D, F)),
            "w_up": _w((lambda *s: _rng.normal(s) * 0.05)(D, F)),
            "w_down": _w((lambda *s: _rng.normal(s) * 0.05)(F, D)),
        }
    _B_in = _B_setup()

    return {
        "A_x": _A_in["x"],
        "A_Lambda_re": _A_in["Lambda_re"],
        "A_Lambda_im": _A_in["Lambda_im"],
        "A_B_re": _A_in["B_re"],
        "A_B_im": _A_in["B_im"],
        "A_C_re": _A_in["C_re"],
        "A_C_im": _A_in["C_im"],
        "A_log_dt": _A_in["log_dt"],
        "A_Dskip": _A_in["Dskip"],
        "B_x": _B_in["x"],
        "B_w_gate": _B_in["w_gate"],
        "B_w_up": _B_in["w_up"],
        "B_w_down": _B_in["w_down"],
    }

def reference(A_x, A_Lambda_re, A_Lambda_im, A_B_re, A_B_im, A_C_re, A_C_im, A_log_dt, A_Dskip, B_x, B_w_gate, B_w_up, B_w_down):
    def _A_ref(x, Lambda_re, Lambda_im, B_re, B_im, C_re, C_im, log_dt, Dskip):
        Bsz, L, H = x.shape
        Lam = Lambda_re + 1j * Lambda_im
        Bmat = B_re + 1j * B_im
        Cmat = C_re + 1j * C_im
        dt = jnp.exp(log_dt)
        Lam_bar = jnp.exp(dt * Lam)
        B_bar = ((Lam_bar - 1.0) / Lam)[:, None] * Bmat
        Bu = jnp.einsum("bld,pd->blp", x + 0j, B_bar)
        h = jnp.zeros_like(Bu[:, 0, :])
        hs = []
        for t in range(L):
            h = Lam_bar[None, :] * h + Bu[:, t, :]
            hs.append(h)
        hseq = jnp.stack(hs, 1)
        y = 2.0 * jnp.einsum("blp,dp->bld", hseq, Cmat).real + x * Dskip[None, None, :]
        return y

    def _B_ref(x, w_gate, w_up, w_down):
        return (_gelu(x @ w_gate) * (x @ w_up)) @ w_down

    x = A_x
    xn = _layernorm(x, axis=-1)
    return x + _A_ref(xn, A_Lambda_re, A_Lambda_im, A_B_re, A_B_im, A_C_re, A_C_im, A_log_dt, A_Dskip) + _B_ref(xn, B_w_gate, B_w_up, B_w_down)
```

```python
import functools
import jax
import jax.numpy as jnp
import numpy as np
from jax import lax
import jax.experimental.pallas as pl
import jax.experimental.pallas.tpu as pltpu

NT = (((1,), (1,)), ((), ()))
NN = (((1,), (0,)), ((), ()))
f32 = jnp.float32
bf16 = jnp.bfloat16
u32 = jnp.uint32

def _gelu(g):
    c = np.float32(np.sqrt(2.0 / np.pi))
    return 0.5 * g * (1.0 + jnp.tanh(c * (g + 0.044715 * (g * g * g))))

def nt(a, b):
    return lax.dot_general(a, b, NT, preferred_element_type=f32)
def nn(a, b):
    return lax.dot_general(a, b, NN, preferred_element_type=f32)

def interleave(gens):
    gens = [[g, w, o] for g, w, o in gens]
    while gens:
        gens.sort(key=lambda e: e[2])
        e = gens[0]
        try:
            next(e[0]); e[2] += 1.0 / e[1]
        except StopIteration:
            gens.pop(0)

def strassen_b(B11, B12, B21, B22):
    return [B11 + B22, B11, B12 - B22, B21 - B11, B22, B11 + B12, B21 + B22]
def strassen_a(A11, A12, A21, A22):
    return [A11 + A22, A21 + A22, A11, A22, A11 + A12, A21 - A11, A12 - A22]
SUMS = (0, 2, 3, 5, 6)
SIDX = {i: j for j, i in enumerate(SUMS)}

class _Null:
    def __enter__(self): return self
    def __exit__(self, *a): return False

def make(T1=256, T2=256, UP=9, scopes=False, RB=16, RC=32, flags=None, order=None,
         sched=None, nsplit=True, chain=1, bsub=1, X0=None, lnch=16, p2only=False, oslots=4, cfirst=False, remfirst=False, scanw=None, reload=False, jit_tg=False, jit_td=False, ploop=0, pace=0):
    L, D, P, F = 2048, 512, 512, 1376
    LH = L // 2
    n2 = LH // T2
    NW = T2 // 2
    HP = NW + 1
    CH = lnch
    xblocks = list(X0 or [])
    while sum(xblocks) < LH: xblocks.append(T1)
    assert sum(xblocks) == LH
    xoff = [sum(xblocks[:i]) for i in range(len(xblocks))]
    n1 = len(xblocks)
    scope = (lambda name: jax.named_scope(name)) if scopes else (lambda name: _Null())

    def kernel(x_hbm, lre_hbm, lim_hbm, bre_hbm, bim_hbm, cre_hbm, cim_hbm, ldt_hbm, dsk_hbm,
               wg_hbm, wu_hbm, wd_hbm, o_hbm,
               x32, vec_v, bre32, bim32, cre32, cim32, wg32, wu32, wd32, sems, osem,
               ab_scr, xs, r_scr, ue, uo, hs, tb, tg, td, tc, as_, arem, o_scr):
        x_v = x32.bitcast(bf16); bre_v = bre32.bitcast(bf16); bim_v = bim32.bitcast(bf16)
        cre_v = cre32.bitcast(bf16); cim_v = cim32.bitcast(bf16)
        wg_v = wg32.bitcast(bf16); wu_v = wu32.bitcast(bf16); wd_v = wd32.bitcast(bf16)
        xs_v = [xs.at[i].bitcast(bf16) for i in range(7)]
        as_v = [as_.at[i].bitcast(bf16) for i in range(7)]
        arem_v = [arem.at[i] for i in range(2)]
        tb_v = [tb.at[i].bitcast(bf16) for i in range(5)]
        tg_v = [tg.at[i].bitcast(bf16) for i in range(5)]
        td_v = [td.at[i].bitcast(bf16) for i in range(5)]
        tc_v = [tc.at[i].bitcast(bf16) for i in range(7)]

        cps = {}
        def add(name, src, dst):
            cps[name] = pltpu.make_async_copy(src, dst, sems.at[len(cps)])
        add("lre", lre_hbm, vec_v.at[0]); add("lim", lim_hbm, vec_v.at[1])
        add("ldt", ldt_hbm, vec_v.at[2]); add("dsk", dsk_hbm, vec_v.at[3])
        for b in range(n1):
            add("x%d" % b, x_hbm.at[pl.ds(2 * xoff[b], 2 * xblocks[b]), :], x_v.at[pl.ds(2 * xoff[b], 2 * xblocks[b]), :])
        add("bre", bre_hbm, bre_v); add("bim", bim_hbm, bim_v)
        add("cre", cre_hbm, cre_v); add("cim", cim_hbm, cim_v)
        add("wg", wg_hbm, wg_v); add("wu", wu_hbm, wu_v); add("wd", wd_hbm, wd_v)
        default_order = ["lre", "lim", "ldt", "dsk", "x0", "bre", "bim"] + ["x%d" % b for b in range(1, n1 - 1)] + ["wg", "wu", "x%d" % (n1 - 1), "cre", "cim", "wd"]
        for k in (order or default_order): cps[k].start()
        waited = set()
        def wait(*names):
            for k in names:
                if k not in waited:
                    cps[k].wait(); waited.add(k)

        wait("lre", "lim", "ldt", "dsk")
        lre = vec_v[0].astype(f32)
        lim = vec_v[1].astype(f32)
        dt = jnp.exp(vec_v[2].astype(f32)).astype(bf16).astype(f32)
        mag = jnp.exp(dt * lre)
        ang = dt * lim
        are = mag * jnp.cos(ang)
        aim = mag * jnp.sin(ang)
        nre = are - 1.0
        den = lre * lre + lim * lim
        ab_scr[0:4, :] = are
        ab_scr[4:8, :] = are
        ab_scr[8:12, :] = -aim
        ab_scr[12:16, :] = aim
        a2re = are * are - aim * aim
        a2im = 2.0 * are * aim
        ab_scr[24:28, :] = a2re
        ab_scr[28:32, :] = a2re
        ab_scr[32:36, :] = -a2im
        ab_scr[36:40, :] = a2im
        ab_scr[16:20, :] = 2.0 * (nre * lre + aim * lim) / den
        ab_scr[20:24, :] = 2.0 * (aim * lre - nre * lim) / den

        def g_ln(blk):
            dsk = vec_v[3].astype(f32)
            zs = []
            for ch in range(xblocks[blk] // CH):
                q0 = xoff[blk] + ch * CH
                w = x32[pl.ds(q0, CH), :]
                if pace and len(zs) >= pace:
                    w = w | zs[-pace]
                xn2 = []
                for par in range(2):
                    if par == 0:
                        x = pltpu.bitcast(w << 16, f32)
                    else:
                        x = pltpu.bitcast(w & jnp.uint32(0xFFFF0000), f32)
                    mu = jnp.sum(x, axis=-1, keepdims=True) * (1.0 / D)
                    xc = x - mu
                    var = jnp.sum(xc * xc, axis=-1, keepdims=True) * (1.0 / D)
                    rs = lax.rsqrt(var + 1e-5)
                    xn = xc * rs
                    if pace and par == 1:
                        zs.append(pltpu.bitcast(jnp.broadcast_to(rs, (CH, 128)), u32) >> 31)
                        zs[-1] = jnp.concatenate([zs[-1]] * 4, axis=1)
                    for c in range(4):
                        sl = slice(c * 128, (c + 1) * 128)
                        r_scr[par, pl.ds(q0, CH), sl] = x[:, sl] + xn[:, sl] * dsk[c:c+1, :]
                    xn2.append(xn)
                S = strassen_a(xn2[0][:, :256], xn2[0][:, 256:], xn2[1][:, :256], xn2[1][:, 256:])
                for i in range(7):
                    xs_v[i][pl.ds(q0, CH), :] = S[i].astype(bf16)
                yield

        def g_tb_():
            for r0 in range(0, 512, RB):
                rows = pl.ds(r0, RB)
                T = strassen_b(bre_v[rows, 0:256].astype(f32), bim_v[rows, 0:256].astype(f32),
                               bre_v[rows, 256:512].astype(f32), bim_v[rows, 256:512].astype(f32))
                for i in SUMS:
                    tb_v[SIDX[i]][rows, :] = T[i].astype(bf16)
                yield

        def g_bmm(blk):
            TS = xblocks[blk] // bsub
            for sub in range(bsub):
                q0 = xoff[blk] + sub * TS
                S = [xs_v[i][pl.ds(q0, TS), :] for i in range(7)]
                for c in range(4):
                    ns = pl.ds(c * 128, 128)
                    T = [tb_v[0][ns, :], bre_v[ns, 0:256], tb_v[1][ns, :], tb_v[2][ns, :],
                         bim_v[ns, 256:512], tb_v[3][ns, :], tb_v[4][ns, :]]
                    M = [nt(S[i], T[i]) for i in range(7)]
                    base = q0 * UP
                    ue[pl.ds(base + c, TS, stride=UP), :] = M[0] + M[3] - M[4] + M[6]
                    ue[pl.ds(base + 4 + c, TS, stride=UP), :] = M[2] + M[4]
                    uo[pl.ds(base + c, TS, stride=UP), :] = M[1] + M[3]
                    uo[pl.ds(base + 4 + c, TS, stride=UP), :] = M[0] - M[1] + M[2] + M[5]
                    yield

        def g_tg_():
            for r0 in range(0, F, RB):
                rows = pl.ds(r0, RB)
                T = strassen_b(wg_v[rows, 0:256].astype(f32), wu_v[rows, 0:256].astype(f32),
                               wg_v[rows, 256:512].astype(f32), wu_v[rows, 256:512].astype(f32))
                for i in SUMS:
                    tg_v[SIDX[i]][rows, :] = T[i].astype(bf16)
                yield

        def g_td_():
            for r0 in range(0, 640, RB):
                T = strassen_b(wd_v[pl.ds(r0, RB), 0:256].astype(f32), wd_v[pl.ds(r0, RB), 256:512].astype(f32),
                               wd_v[pl.ds(640 + r0, RB), 0:256].astype(f32), wd_v[pl.ds(640 + r0, RB), 256:512].astype(f32))
                for i in SUMS:
                    td_v[SIDX[i]][pl.ds(r0, RB), :] = T[i].astype(bf16)
                yield

        def g_tc_():
            cre = ab_scr[16:20, :]
            cim = ab_scr[20:24, :]
            for r0 in range(0, 256, RC):
                for c in range(4):
                    sl = slice(c * 128, (c + 1) * 128)
                    rr = cre[c:c+1, :]
                    mm = cim[c:c+1, :]
                    q = []
                    for dh in range(2):
                        rows = pl.ds(dh * 256 + r0, RC)
                        Cre = cre_v[rows, sl].astype(f32)
                        Cim = cim_v[rows, sl].astype(f32)
                        q.append((Cre * rr - Cim * mm, Cre * mm + Cim * rr))
                    Re0, Im0 = q[0]; Re1, Im1 = q[1]
                    T = [Re0 - Im1, Re0, Re1 + Im1, -(Im0 + Re0), -Im1, Re0 + Re1, Im0 + Im1]
                    for i in range(7):
                        tc_v[i][pl.ds(r0, RC), sl] = T[i].astype(bf16)
                yield

        def presum_loop(nrows, srcs, dsts, step):
            def body(k, c):
                for u_ in range(step // 16):
                    r0 = pl.multiple_of(k * step + u_ * 16, 16)
                    q = [ref[pl.ds(ro + r0, 16), cs_].astype(f32) for (ref, ro, cs_) in srcs]
                    T = strassen_b(*q)
                    for i in SUMS:
                        dsts[SIDX[i]][pl.ds(r0, 16), :] = T[i].astype(bf16)
                return c
            lax.fori_loop(0, nrows // step, body, 0)
        lo, hi = slice(0, 256), slice(256, 512)
        def l_tb():
            presum_loop(512, [(bre_v, 0, lo), (bim_v, 0, lo), (bre_v, 0, hi), (bim_v, 0, hi)], tb_v, ploop); yield
        def l_tg():
            presum_loop(F, [(wg_v, 0, lo), (wu_v, 0, lo), (wg_v, 0, hi), (wu_v, 0, hi)], tg_v, 32); yield
        def l_td():
            presum_loop(640, [(wd_v, 0, lo), (wd_v, 0, hi), (wd_v, 640, lo), (wd_v, 640, hi)], td_v, ploop); yield
        def l_tc():
            cre = ab_scr[16:20, :]
            cim = ab_scr[20:24, :]
            def body(k, carry):
                r0 = pl.multiple_of(k * 16, 16)
                for c in range(4):
                    sl = slice(c * 128, (c + 1) * 128)
                    rr = cre[c:c+1, :]
                    mm = cim[c:c+1, :]
                    q = []
                    for dh in range(2):
                        rows = pl.ds(dh * 256 + r0, 16)
                        Cre = cre_v[rows, sl].astype(f32)
                        Cim = cim_v[rows, sl].astype(f32)
                        q.append((Cre * rr - Cim * mm, Cre * mm + Cim * rr))
                    Re0, Im0 = q[0]; Re1, Im1 = q[1]
                    T = [Re0 - Im1, Re0, Re1 + Im1, -(Im0 + Re0), -Im1, Re0 + Re1, Im0 + Im1]
                    for i in range(7):
                        tc_v[i][pl.ds(r0, 16), sl] = T[i].astype(bf16)
                return carry
            lax.fori_loop(0, 16, body, 0); yield
        g_tb, g_tg, g_td, g_tc = (l_tb, l_tg, l_td, l_tc) if ploop else (g_tb_, g_tg_, g_td_, g_tc_)

        tasks = dict(tg=(g_tg, F // RB, ("wg", "wu")), td=(g_td, 640 // RB, ("wd",)), tc=(g_tc, 256 // RC, ("cre", "cim")))
        the_sched = sched if sched is not None else {n1 - 1: ["tg"], n1: ["tc", "td"]}

        if p2only:
            wait(*cps.keys())
            xs[...] = jnp.zeros_like(xs); tg[...] = jnp.zeros_like(tg); td[...] = jnp.zeros_like(td); tc[...] = jnp.zeros_like(tc)
            ue[...] = jnp.zeros_like(ue); uo[...] = jnp.zeros_like(uo); r_scr[...] = jnp.zeros_like(r_scr)
        with scope("x0w"):
            wait("x0")
        with scope("ln0"):
            for _ in (g_ln(0) if not p2only else []): pass
        with scope("bw"):
            wait("bre", "bim")
        with scope("tb"):
            for _ in (g_tb() if not p2only else []): pass

        for blk in range(n1 if not p2only else 0):
            with scope("p1_%d" % blk):
                gens = [(g_bmm(blk), 4 * bsub, 0.0)]
                if blk + 1 < n1:
                    wait("x%d" % (blk + 1))
                    gens.append((g_ln(blk + 1), xblocks[blk + 1] // CH, 0.001))
                for t in the_sched.get(blk, []):
                    wait(*tasks[t][2])
                    gens.append((tasks[t][0](), tasks[t][1], 0.002))
                interleave(gens)
        with scope("mid"):
            for t in (the_sched.get(n1, []) if not p2only else []):
                wait(*tasks[t][2])
                for _ in tasks[t][0](): pass
            wait("wg", "wu", "wd", "cre", "cim")

        def ocopy(n, slot, c):
            return pltpu.make_async_copy(o_scr.at[slot, c, pl.ds(0, 2 * T2), :],
                                         o_hbm.at[pl.ds(n * 2 * T2, 2 * T2), pl.ds(c * 128, 128)], osem.at[slot * 4 + c])

        top = lax.broadcasted_iota(jnp.int32, (8, 128), 0) < 4

        def phase2(n, h):
            slot = n % oslots
            hcell = [h]
            q0 = pl.multiple_of(n * T2, T2)

            if oslots < n2:
                @pl.when(n >= oslots)
                def _():
                    for c in range(4):
                        ocopy(n - oslots, slot, c).wait()

            def g_scan():
                A = ab_scr[0:8, :]
                Bm = ab_scr[8:16, :]
                A2 = ab_scr[24:32, :]
                B2 = ab_scr[32:40, :]
                h = hcell[0]
                sh = pltpu.roll(h, 4, 0)
                base = pl.multiple_of(n * (T2 * UP), T2 * UP)
                for w in range(NW):
                    parts = []
                    for k in range(2):
                        q = 2 * w + k
                        if chain == 2:
                            u0 = ue[pl.ds(base + q * UP, 8), :]
                            u1 = uo[pl.ds(base + q * UP, 8), :]
                            v = (A * u0 + u1) + Bm * pltpu.roll(u0, 4, 0)
                            h0 = (A * h + u0) + Bm * sh
                            h = (A2 * h + v) + B2 * sh
                            sh0 = pltpu.roll(h0, 4, 0)
                        elif chain == 0:
                            h0 = A * h + Bm * sh + ue[pl.ds(base + q * UP, 8), :]
                            sh0 = pltpu.roll(h0, 4, 0)
                            h = A * h0 + Bm * sh0 + uo[pl.ds(base + q * UP, 8), :]
                        else:
                            h0 = (A * h + ue[pl.ds(base + q * UP, 8), :]) + Bm * sh
                            sh0 = pltpu.roll(h0, 4, 0)
                            h = (A * h0 + uo[pl.ds(base + q * UP, 8), :]) + Bm * sh0
                        sh = pltpu.roll(h, 4, 0)
                        X = jnp.where(top, h0, h)
                        parts.append((X, X + sh, h - h0, h0 + sh0))
                    for j in range(4):
                        wd_ = pltpu.pack_elementwise([parts[0][j], parts[1][j]], packed_dtype=bf16)
                        hs[pl.ds(j * 8 * HP + w, 8, stride=HP), :] = wd_
                    yield
                hcell[0] = h

            avals = {}
            def g_gu():
                S = [xs_v[i][pl.ds(q0, T2), :] for i in range(7)]
                def tile(j0, jw):
                    ns = pl.ds(j0, jw)
                    if jit_tg:
                        raw = [wg_v[ns, 0:256], wu_v[ns, 0:256], wg_v[ns, 256:512], wu_v[ns, 256:512]]
                        Tf = strassen_b(*[q_.astype(f32) for q_ in raw])
                        T = [raw[0] if i == 1 else raw[3] if i == 4 else Tf[i].astype(bf16) for i in range(7)]
                    else:
                        T = [tg_v[0][ns, :], wg_v[ns, 0:256], tg_v[1][ns, :], tg_v[2][ns, :],
                             wu_v[ns, 256:512], tg_v[3][ns, :], tg_v[4][ns, :]]
                    M = [nt(S[i], T[i]) for i in range(7)]
                    ge = M[0] + M[3] - M[4] + M[6]
                    ue_ = M[2] + M[4]
                    go = M[1] + M[3]
                    uo_ = M[0] - M[1] + M[2] + M[5]
                    return _gelu(ge) * ue_, _gelu(go) * uo_
                for j in range(5):
                    A11, A21 = tile(j * 128, 128)
                    yield
                    A12, A22 = tile(640 + j * 128, 128)
                    SS = strassen_a(A11, A12, A21, A22)
                    for i in range(7):
                        as_v[i][:, j * 128:(j + 1) * 128] = SS[i].astype(bf16)
                    yield
                ae, ao = tile(1280, 96)
                arem_v[0][...] = ae.astype(bf16)
                arem_v[1][...] = ao.astype(bf16)
                yield

            interleave([(g_gu(), 11, 0.0), (g_scan(), scanw or NW, 0.001)])

            def hs_mat(slab0):
                return jnp.concatenate([pltpu.bitcast(hs[pl.ds((slab0 + c) * HP, NW), :], bf16) for c in range(4)], axis=1)
            slab = [8, 12, 0, 4, 24, 16, 20]
            AS = [as_v[i][...] for i in range(7)]
            HS = [hs_mat(slab[i]) for i in range(7)]
            are_, aro_ = arem_v[0][...], arem_v[1][...]
            halves = [(0, 128), (128, 128)] if nsplit else [(0, 256)]
            Mc = {}
            if cfirst:
                for (c0, cw) in halves[:1]:
                    for i in range(7):
                        Mc[(c0, i)] = nt(HS[i], tc_v[i][pl.ds(c0, cw), :])
            for (c0, cw) in halves:
                cs = pl.ds(c0, cw)
                if cfirst and (c0, 0) not in Mc:
                    for i in range(7):
                        Mc[(c0, i)] = nt(HS[i], tc_v[i][pl.ds(c0, cw), :])
                M = []
                if jit_td:
                    raw = [wd_v[0:640, cs], wd_v[0:640, pl.ds(256 + c0, cw)], wd_v[640:1280, cs], wd_v[640:1280, pl.ds(256 + c0, cw)]]
                    TDj = [t_.astype(bf16) for t_ in strassen_b(*[q_.astype(f32) for q_ in raw])]
                for i in range(7):
                    if i == 1:
                        Ti = wd_v[0:640, cs]
                    elif i == 4:
                        Ti = wd_v[640:1280, pl.ds(256 + c0, cw)]
                    elif jit_td:
                        Ti = TDj[i]
                    else:
                        Ti = td_v[SIDX[i]][:, cs]
                    if reload:
                        AS[i] = as_v[i][...]; HS[i] = hs_mat(slab[i])
                    if cfirst:
                        M.append(Mc[(c0, i)] + nn(AS[i], Ti))
                    else:
                        M.append(nn(AS[i], Ti) + nt(HS[i], tc_v[i][cs, :]))
                outs = [(0, 0, M[0] + M[3] - M[4] + M[6]), (0, 256, M[2] + M[4]),
                        (1, 0, M[1] + M[3]), (1, 256, M[0] - M[1] + M[2] + M[5])]
                for par, cb, y in outs:
                    cols = pl.ds(cb + c0, cw)
                    y = y + nn(are_ if par == 0 else aro_, wd_v[1280:1376, cols]) + r_scr[par, pl.ds(q0, T2), cols]
                    for k in range(cw // 128):
                        o_scr[slot, (cb + c0) // 128 + k, pl.ds(par, T2, stride=2), :] = y[:, k * 128:(k + 1) * 128]
                for cb in (0, 256):
                    for k in range(cw // 128):
                        ocopy(n, slot, (cb + c0) // 128 + k).start()
            return hcell[0]

        with scope("ph2"):
            lax.fori_loop(0, n2, phase2, jnp.zeros((8, 128), f32))
        with scope("tail"):
            for nn_ in range(max(0, n2 - oslots), n2):
                for c in range(4):
                    ocopy(nn_, nn_ % oslots, c).wait()

    anyspec = pl.BlockSpec(memory_space=pltpu.HBM)
    V = pltpu.VMEM
    call = pl.pallas_call(
        kernel,
        in_specs=[anyspec] * 12,
        out_specs=anyspec,
        out_shape=jax.ShapeDtypeStruct((L, D), f32),
        scratch_shapes=[V((L // 2, D), u32), V((4, 4, 128), bf16),
                        V((P // 2, D), u32), V((P // 2, D), u32), V((D // 2, P), u32), V((D // 2, P), u32),
                        V((F // 2, D), u32), V((F // 2, D), u32), V((F // 2, D), u32),
                        pltpu.SemaphoreType.DMA((11 + n1,)), pltpu.SemaphoreType.DMA((4 * oslots,)),
                        V((40, 128), f32),
                        V((7, LH // 2, 256), u32),
                        V((2, LH, D), f32),
                        V((LH * UP + 8, 128), f32), V((LH * UP + 8, 128), f32),
                        V((32 * HP + 8, 128), u32),
                        V((5, 256, 256), u32),
                        V((5, F // 2, 256), u32),
                        V((5, 320, 256), u32),
                        V((7, 128, 512), u32),
                        V((7, T2 // 2, 640), u32),
                        V((2, T2, 96), bf16),
                        V((oslots, 4, 2 * T2 + 8, 128), f32)],
        compiler_params=pltpu.CompilerParams(vmem_limit_bytes=110 * 1024 * 1024, flags=flags),
        name="ssm_geglu_strassen",
    )

    @jax.jit
    def fn(A_x, A_Lambda_re, A_Lambda_im, A_B_re, A_B_im, A_C_re, A_C_im, A_log_dt, A_Dskip, B_x, B_w_gate, B_w_up, B_w_down):
        r = lambda v: v.reshape(4, 128)
        out = call(A_x.reshape(L, D), r(A_Lambda_re), r(A_Lambda_im), A_B_re, A_B_im, A_C_re, A_C_im,
                   r(A_log_dt), r(A_Dskip), B_w_gate.T, B_w_up.T, B_w_down)
        return out.reshape(1, L, D)
    return fn


pallas_parallel_sum__ssm_conv_s5__geglu_ffn__prompt_kernel = make(
    nsplit=True, flags={"XLA_TPU_EVENLY_DISTRIBUTE_CRITICAL_NODES": True})
```

```python
import functools
import jax
import jax.numpy as jnp
import numpy as np
from jax import lax
import jax.experimental.pallas as pl
import jax.experimental.pallas.tpu as pltpu

NT = (((1,), (1,)), ((), ()))
NN = (((1,), (0,)), ((), ()))
f32 = jnp.float32
bf16 = jnp.bfloat16
u32 = jnp.uint32

def _gelu(g):
    c = np.float32(np.sqrt(2.0 / np.pi))
    return 0.5 * g * (1.0 + jnp.tanh(c * (g + 0.044715 * (g * g * g))))

def nt(a, b):
    return lax.dot_general(a, b, NT, preferred_element_type=f32)
def nn(a, b):
    return lax.dot_general(a, b, NN, preferred_element_type=f32)

def interleave(gens):
    gens = [[g, w, o] for g, w, o in gens]
    while gens:
        gens.sort(key=lambda e: e[2])
        e = gens[0]
        try:
            next(e[0]); e[2] += 1.0 / e[1]
        except StopIteration:
            gens.pop(0)

def strassen_b(B11, B12, B21, B22):
    return [B11 + B22, B11, B12 - B22, B21 - B11, B22, B11 + B12, B21 + B22]
def strassen_a(A11, A12, A21, A22):
    return [A11 + A22, A21 + A22, A11, A22, A11 + A12, A21 - A11, A12 - A22]
SUMS = (0, 2, 3, 5, 6)
SIDX = {i: j for j, i in enumerate(SUMS)}

class _Null:
    def __enter__(self): return self
    def __exit__(self, *a): return False

def make(T1=256, T2=256, UP=9, scopes=False, RB=16, RC=32, flags=None, order=None,
         sched=None, nsplit=True, chain=1, bsub=1, X0=None, lnch=16, p2only=False, oslots=4, cfirst=False, remfirst=False, scanw=None, reload=False, jit_tg=False, jit_td=False, ploop=0, pace=0, gusub=1, porder=None, gform=0, nor=True, pd=None, plan=None):
    L, D, P, F = 2048, 512, 512, 1376
    LH = L // 2
    n2 = LH // T2
    NW = T2 // 2
    HP = NW + 1
    CH = lnch
    xblocks = list(X0 or [])
    while sum(xblocks) < LH: xblocks.append(T1)
    assert sum(xblocks) == LH
    xoff = [sum(xblocks[:i]) for i in range(len(xblocks))]
    n1 = len(xblocks)
    scope = (lambda name: jax.named_scope(name)) if scopes else (lambda name: _Null())

    def kernel(x_hbm, lre_hbm, lim_hbm, bre_hbm, bim_hbm, cre_hbm, cim_hbm, ldt_hbm, dsk_hbm,
               wg_hbm, wu_hbm, wd_hbm, o_hbm,
               x32, vec_v, bre32, bim32, cre32, cim32, wg32, wu32, wd32, sems, osem,
               ab_scr, xs, r_scr, ue, uo, hs, tb, tg, td, tc, as_, arem, o_scr, xnp):
        x_v = x32.bitcast(bf16); bre_v = bre32.bitcast(bf16); bim_v = bim32.bitcast(bf16)
        cre_v = cre32.bitcast(bf16); cim_v = cim32.bitcast(bf16)
        wg_v = wg32.bitcast(bf16); wu_v = wu32.bitcast(bf16); wd_v = wd32.bitcast(bf16)
        xs_v = [xs.at[i].bitcast(bf16) for i in range(7)]
        as_v = [as_.at[i].bitcast(bf16) for i in range(7)]
        arem_v = [arem.at[i] for i in range(2)]
        tb_v = [tb.at[i].bitcast(bf16) for i in range(5)]
        tg_v = [tg.at[i].bitcast(bf16) for i in range(5)]
        td_v = [td.at[i].bitcast(bf16) for i in range(5)]
        tc_v = [tc.at[i].bitcast(bf16) for i in range(7)]

        cps = {}
        def add(name, src, dst):
            cps[name] = pltpu.make_async_copy(src, dst, sems.at[len(cps)])
        add("lre", lre_hbm, vec_v.at[0]); add("lim", lim_hbm, vec_v.at[1])
        add("ldt", ldt_hbm, vec_v.at[2]); add("dsk", dsk_hbm, vec_v.at[3])
        for b in range(n1):
            add("x%d" % b, x_hbm.at[pl.ds(2 * xoff[b], 2 * xblocks[b]), :], x_v.at[pl.ds(2 * xoff[b], 2 * xblocks[b]), :])
        for hh_ in range(2):
            add("bre%d" % hh_, bre_hbm.at[pl.ds(hh_ * 256, 256), :], bre_v.at[pl.ds(hh_ * 256, 256), :])
            add("bim%d" % hh_, bim_hbm.at[pl.ds(hh_ * 256, 256), :], bim_v.at[pl.ds(hh_ * 256, 256), :])
        add("cre", cre_hbm, cre_v); add("cim", cim_hbm, cim_v)
        add("wg", wg_hbm, wg_v); add("wu", wu_hbm, wu_v); add("wd", wd_hbm, wd_v)
        alias = dict(b0=["bre0", "bim0"], b1=["bre1", "bim1"], c=["cre", "cim"], w=["wg", "wu"])
        def expand(names):
            out = []
            for k in names: out += alias.get(k, [k])
            return out
        full_order = ["lre", "lim", "ldt", "dsk"] + expand(order)
        assert sorted(full_order) == sorted(cps), (full_order, list(cps))
        for k in full_order: cps[k].start()
        waited = set()
        def wait(*names):
            for k in expand(names):
                if k not in waited:
                    cps[k].wait(); waited.add(k)

        wait("lre", "lim", "ldt", "dsk")
        lre = vec_v[0].astype(f32)
        lim = vec_v[1].astype(f32)
        dt = jnp.exp(vec_v[2].astype(f32)).astype(bf16).astype(f32)
        mag = jnp.exp(dt * lre)
        ang = dt * lim
        are = mag * jnp.cos(ang)
        aim = mag * jnp.sin(ang)
        nre = are - 1.0
        den = lre * lre + lim * lim
        ab_scr[0:4, :] = are
        ab_scr[4:8, :] = are
        ab_scr[8:12, :] = -aim
        ab_scr[12:16, :] = aim
        a2re = are * are - aim * aim
        a2im = 2.0 * are * aim
        ab_scr[24:28, :] = a2re
        ab_scr[28:32, :] = a2re
        ab_scr[32:36, :] = -a2im
        ab_scr[36:40, :] = a2im
        ab_scr[16:20, :] = 2.0 * (nre * lre + aim * lim) / den
        ab_scr[20:24, :] = 2.0 * (aim * lre - nre * lim) / den

        zcell = [0]
        def new_zero(ref):
            wv = ref[0:8, 0:128]
            zcell[0] = jnp.sum(jnp.minimum((wv >> 31).astype(jnp.int32), 0))
        def pacer(n, delay, start=0):
            out = []
            zop = zcell[0]
            sv = zop
            for _ in range(start):
                sv = sv + zop
            for k_ in range(n):
                out.append(sv)
                for j_ in range(delay):
                    sv = (sv + zop) if j_ % 2 == 0 else (sv | zop)
            return out

        def g_ln(blk, pd_=None):
            dsk = vec_v[3].astype(f32)
            zs = []
            pz = pacer(xblocks[blk] // CH, *pd_) if pd_ else None
            for ch in range(xblocks[blk] // CH):
                q0 = xoff[blk] + ch * CH
                w = x32[pl.ds(pl.multiple_of(q0 + pz[ch], CH) if pz else q0, CH), :]
                if pace and len(zs) >= pace:
                    w = w | zs[-pace]
                xn2 = []
                for par in range(2):
                    if par == 0:
                        x = pltpu.bitcast(w << 16, f32)
                    else:
                        x = pltpu.bitcast(w & jnp.uint32(0xFFFF0000), f32)
                    mu = jnp.sum(x, axis=-1, keepdims=True) * (1.0 / D)
                    xc = x - mu
                    var = jnp.sum(xc * xc, axis=-1, keepdims=True) * (1.0 / D)
                    rs = lax.rsqrt(var + 1e-5)
                    xn = xc * rs
                    if pace and par == 1:
                        zs.append(pltpu.bitcast(jnp.broadcast_to(rs, (CH, 128)), u32) >> 31)
                        zs[-1] = jnp.concatenate([zs[-1]] * 4, axis=1)
                    if not nor:
                        for c in range(4):
                            sl = slice(c * 128, (c + 1) * 128)
                            r_scr[par, pl.ds(q0, CH), sl] = x[:, sl] + xn[:, sl] * dsk[c:c+1, :]
                    xn2.append(xn)
                if nor:
                    xnp[pl.ds(q0, CH), :] = pltpu.pack_elementwise(xn2, packed_dtype=bf16)
                S = strassen_a(xn2[0][:, :256], xn2[0][:, 256:], xn2[1][:, :256], xn2[1][:, 256:])
                for i in range(7):
                    xs_v[i][pl.ds(q0, CH), :] = S[i].astype(bf16)
                yield

        def g_tb_(pd_=None, lo_=0, hi_=512):
            pz = pacer((hi_ - lo_) // RB, *pd_) if pd_ else None
            for r0 in range(lo_, hi_, RB):
                rows = pl.ds(r0, RB)
                rl = pl.ds(pl.multiple_of(r0 + pz[(r0 - lo_) // RB], RB), RB) if pz else rows
                T = strassen_b(bre_v[rl, 0:256].astype(f32), bim_v[rl, 0:256].astype(f32),
                               bre_v[rl, 256:512].astype(f32), bim_v[rl, 256:512].astype(f32))
                for i in SUMS:
                    tb_v[SIDX[i]][rows, :] = T[i].astype(bf16)
                yield

        def g_bmm(qq, TT, tiles):
            TS = TT // bsub
            for sub in range(bsub):
                q0 = qq + sub * TS
                S = [xs_v[i][pl.ds(q0, TS), :] for i in range(7)]
                for c in tiles:
                    ns = pl.ds(c * 128, 128)
                    T = [tb_v[0][ns, :], bre_v[ns, 0:256], tb_v[1][ns, :], tb_v[2][ns, :],
                         bim_v[ns, 256:512], tb_v[3][ns, :], tb_v[4][ns, :]]
                    M = [nt(S[i], T[i]) for i in range(7)]
                    base = q0 * UP
                    ue[pl.ds(base + c, TS, stride=UP), :] = M[0] + M[3] - M[4] + M[6]
                    ue[pl.ds(base + 4 + c, TS, stride=UP), :] = M[2] + M[4]
                    uo[pl.ds(base + c, TS, stride=UP), :] = M[1] + M[3]
                    uo[pl.ds(base + 4 + c, TS, stride=UP), :] = M[0] - M[1] + M[2] + M[5]
                    yield

        def g_tg_(pd_=None, lo_=0, hi_=F):
            pz = pacer((hi_ - lo_) // RB, *pd_) if pd_ else None
            for r0 in range(lo_, hi_, RB):
                rows = pl.ds(r0, RB)
                rl = pl.ds(pl.multiple_of(r0 + pz[(r0 - lo_) // RB], RB), RB) if pz else rows
                T = strassen_b(wg_v[rl, 0:256].astype(f32), wu_v[rl, 0:256].astype(f32),
                               wg_v[rl, 256:512].astype(f32), wu_v[rl, 256:512].astype(f32))
                for i in SUMS:
                    tg_v[SIDX[i]][rows, :] = T[i].astype(bf16)
                yield

        def g_td_(pd_=None):
            pz = pacer(640 // RB, *pd_) if pd_ else None
            for r0 in range(0, 640, RB):
                rr0 = pl.multiple_of(r0 + pz[r0 // RB], RB) if pz else r0
                T = strassen_b(wd_v[pl.ds(rr0, RB), 0:256].astype(f32), wd_v[pl.ds(rr0, RB), 256:512].astype(f32),
                               wd_v[pl.ds(640 + rr0, RB), 0:256].astype(f32), wd_v[pl.ds(640 + rr0, RB), 256:512].astype(f32))
                for i in SUMS:
                    td_v[SIDX[i]][pl.ds(r0, RB), :] = T[i].astype(bf16)
                yield

        def g_tc_(pd_=None):
            cre = ab_scr[16:20, :]
            cim = ab_scr[20:24, :]
            pz = pacer(4 * 256 // RC, *pd_) if pd_ else None
            for r0 in range(0, 256, RC):
                for c in range(4):
                    sl = slice(c * 128, (c + 1) * 128)
                    rr = cre[c:c+1, :]
                    mm = cim[c:c+1, :]
                    q = []
                    for dh in range(2):
                        rows = pl.ds(pl.multiple_of(dh * 256 + r0 + pz[(r0 // RC) * 4 + c], RC) if pz else dh * 256 + r0, RC)
                        Cre = cre_v[rows, sl].astype(f32)
                        Cim = cim_v[rows, sl].astype(f32)
                        q.append((Cre * rr - Cim * mm, Cre * mm + Cim * rr))
                    Re0, Im0 = q[0]; Re1, Im1 = q[1]
                    T = [Re0 - Im1, Re0, Re1 + Im1, -(Im0 + Re0), -Im1, Re0 + Re1, Im0 + Im1]
                    for i in range(7):
                        tc_v[i][pl.ds(r0, RC), sl] = T[i].astype(bf16)
                yield

        def presum_loop(nrows, srcs, dsts, step):
            def body(k, c):
                for u_ in range(step // 16):
                    r0 = pl.multiple_of(k * step + u_ * 16, 16)
                    q = [ref[pl.ds(ro + r0, 16), cs_].astype(f32) for (ref, ro, cs_) in srcs]
                    T = strassen_b(*q)
                    for i in SUMS:
                        dsts[SIDX[i]][pl.ds(r0, 16), :] = T[i].astype(bf16)
                return c
            lax.fori_loop(0, nrows // step, body, 0)
        lo, hi = slice(0, 256), slice(256, 512)
        def l_tb():
            presum_loop(512, [(bre_v, 0, lo), (bim_v, 0, lo), (bre_v, 0, hi), (bim_v, 0, hi)], tb_v, ploop); yield
        def l_tg():
            presum_loop(F, [(wg_v, 0, lo), (wu_v, 0, lo), (wg_v, 0, hi), (wu_v, 0, hi)], tg_v, 32); yield
        def l_td():
            presum_loop(640, [(wd_v, 0, lo), (wd_v, 0, hi), (wd_v, 640, lo), (wd_v, 640, hi)], td_v, ploop); yield
        def l_tc():
            cre = ab_scr[16:20, :]
            cim = ab_scr[20:24, :]
            def body(k, carry):
                r0 = pl.multiple_of(k * 16, 16)
                for c in range(4):
                    sl = slice(c * 128, (c + 1) * 128)
                    rr = cre[c:c+1, :]
                    mm = cim[c:c+1, :]
                    q = []
                    for dh in range(2):
                        rows = pl.ds(dh * 256 + r0, 16)
                        Cre = cre_v[rows, sl].astype(f32)
                        Cim = cim_v[rows, sl].astype(f32)
                        q.append((Cre * rr - Cim * mm, Cre * mm + Cim * rr))
                    Re0, Im0 = q[0]; Re1, Im1 = q[1]
                    T = [Re0 - Im1, Re0, Re1 + Im1, -(Im0 + Re0), -Im1, Re0 + Re1, Im0 + Im1]
                    for i in range(7):
                        tc_v[i][pl.ds(r0, 16), sl] = T[i].astype(bf16)
                return carry
            lax.fori_loop(0, 16, body, 0); yield
        g_tb, g_tg, g_td, g_tc = (l_tb, l_tg, l_td, l_tc) if ploop else (g_tb_, g_tg_, g_td_, g_tc_)

        tasks = dict(tg=(g_tg, F // RB, ("wg", "wu")), td=(g_td, 640 // RB, ("wd",)), tc=(g_tc, 256 // RC, ("cre", "cim")),
                     tga=(lambda p_=None: g_tg_(p_, 0, 688), 43, ("wg", "wu")), tgb=(lambda p_=None: g_tg_(p_, 688, F), 43, ("wg", "wu")))


        if p2only:
            wait(*cps.keys())
            xs[...] = jnp.zeros_like(xs); tg[...] = jnp.zeros_like(tg); td[...] = jnp.zeros_like(td); tc[...] = jnp.zeros_like(tc)
            ue[...] = jnp.zeros_like(ue); uo[...] = jnp.zeros_like(uo); r_scr[...] = jnp.zeros_like(r_scr)
        zsrc = dict(b0=bre32, b1=bre32.at[pl.ds(128, 8)], c=cre32, w=wg32, wd=wd32)
        for b_ in range(n1): zsrc["x%d" % b_] = x32.at[pl.ds(xoff[b_], 8)]
        for si, (waits, tl) in enumerate(plan if not p2only else []):
            with scope("s%d" % si):
                wait(*waits)
                if waits: new_zero(zsrc[waits[-1]])
                gens = []
                for ti, t in enumerate(tl):
                    if t[0] == "b":
                        gens.append((g_bmm(t[1], t[2], t[3]), len(t[3]) * bsub, 0.0))
                    elif t[0] == "ln":
                        gens.append((g_ln(t[1], t[2]), xblocks[t[1]] // CH, 0.001))
                    elif t[0] == "tb":
                        gens.append((g_tb_(t[1], t[2], t[3]), 16, 0.002))
                    elif t[0] == "tg":
                        gens.append((g_tg_(t[1], *t[2:]), 43, 0.002))
                    elif t[0] == "td":
                        gens.append((g_td_(t[1]), 40, 0.002))
                    elif t[0] == "tc":
                        gens.append((g_tc_(t[1]), 8, 0.002))
                interleave(gens)
        wait(*[k for k in cps])

        def ocopy(n, slot, c):
            return pltpu.make_async_copy(o_scr.at[slot, c, pl.ds(0, 2 * T2), :],
                                         o_hbm.at[pl.ds(n * 2 * T2, 2 * T2), pl.ds(c * 128, 128)], osem.at[slot * 4 + c])

        top = lax.broadcasted_iota(jnp.int32, (8, 128), 0) < 4

        def phase2(n, h):
            slot = n % oslots
            hcell = [h]
            q0 = pl.multiple_of(n * T2, T2)

            if oslots < n2:
                @pl.when(n >= oslots)
                def _():
                    for c in range(4):
                        ocopy(n - oslots, slot, c).wait()

            def g_scan():
                A = ab_scr[0:8, :]
                Bm = ab_scr[8:16, :]
                A2 = ab_scr[24:32, :]
                B2 = ab_scr[32:40, :]
                h = hcell[0]
                sh = pltpu.roll(h, 4, 0)
                base = pl.multiple_of(n * (T2 * UP), T2 * UP)
                parts = []
                pend = None
                for w in range(NW):
                    if chain != 3: parts = []
                    for k in range(2):
                        q = 2 * w + k
                        if chain == 3:
                            t1 = A * h
                            z = t1 * 0.0
                            if q > 0:
                                Xp, shp, h1p, h0p, sh0p, z0p = pend
                                parts.append((Xp, (Xp + z) + shp, h1p - h0p, (h0p + z0p) + sh0p))
                            h0 = (t1 + ue[pl.ds(base + q * UP, 8), :]) + (Bm + z) * sh
                            sh0 = pltpu.roll(h0, 4, 0)
                            t1 = A * h0
                            z0 = t1 * 0.0
                            h = (t1 + uo[pl.ds(base + q * UP, 8), :]) + (Bm + z0) * sh0
                            sh = pltpu.roll(h, 4, 0)
                            pend = (jnp.where(top, h0, h), sh, h, h0, sh0, z0)
                            if len(parts) == 2:
                                for j in range(4):
                                    wd_ = pltpu.pack_elementwise([parts[0][j], parts[1][j]], packed_dtype=bf16)
                                    hs[pl.ds(j * 8 * HP + (q // 2 - 1), 8, stride=HP), :] = wd_
                                parts = []
                            continue
                        if chain == 2:
                            u0 = ue[pl.ds(base + q * UP, 8), :]
                            u1 = uo[pl.ds(base + q * UP, 8), :]
                            v = (A * u0 + u1) + Bm * pltpu.roll(u0, 4, 0)
                            h0 = (A * h + u0) + Bm * sh
                            h = (A2 * h + v) + B2 * sh
                            sh0 = pltpu.roll(h0, 4, 0)
                        elif chain == 0:
                            h0 = A * h + Bm * sh + ue[pl.ds(base + q * UP, 8), :]
                            sh0 = pltpu.roll(h0, 4, 0)
                            h = A * h0 + Bm * sh0 + uo[pl.ds(base + q * UP, 8), :]
                        else:
                            h0 = (A * h + ue[pl.ds(base + q * UP, 8), :]) + Bm * sh
                            sh0 = pltpu.roll(h0, 4, 0)
                            h = (A * h0 + uo[pl.ds(base + q * UP, 8), :]) + Bm * sh0
                        sh = pltpu.roll(h, 4, 0)
                        X = jnp.where(top, h0, h)
                        parts.append((X, X + sh, h - h0, h0 + sh0))
                    if chain != 3:
                        for j in range(4):
                            wd_ = pltpu.pack_elementwise([parts[0][j], parts[1][j]], packed_dtype=bf16)
                            hs[pl.ds(j * 8 * HP + w, 8, stride=HP), :] = wd_
                    yield
                if chain == 3:
                    Xp, shp, h1p, h0p, sh0p, z0p = pend
                    parts.append((Xp, Xp + shp, h1p - h0p, (h0p + z0p) + sh0p))
                    for j in range(4):
                        wd_ = pltpu.pack_elementwise([parts[0][j], parts[1][j]], packed_dtype=bf16)
                        hs[pl.ds(j * 8 * HP + NW - 1, 8, stride=HP), :] = wd_
                hcell[0] = h

            avals = {}
            def g_gu():
                TS = T2 // gusub
                def tile(S, j0, jw):
                    ns = pl.ds(j0, jw)
                    T = [tg_v[0][ns, :], wg_v[ns, 0:256], tg_v[1][ns, :], tg_v[2][ns, :],
                         wu_v[ns, 256:512], tg_v[3][ns, :], tg_v[4][ns, :]]
                    M = [None] * 7
                    for i in (porder or range(7)):
                        M[i] = nt(S[i], T[i])
                    if gform == 0:
                        ge = M[0] + M[3] - M[4] + M[6]
                        uo_ = M[0] - M[1] + M[2] + M[5]
                    else:
                        ge = (M[0] + M[3]) + (M[6] - M[4])
                        uo_ = (M[0] - M[1]) + (M[2] + M[5])
                    ue_ = M[2] + M[4]
                    go = M[1] + M[3]
                    return _gelu(ge) * ue_, _gelu(go) * uo_
                Ss = [[xs_v[i][pl.ds(q0 + sb * TS, TS), :] for i in range(7)] for sb in range(gusub)]
                def rem():
                    for sb in range(gusub):
                        ae, ao = tile(Ss[sb], 1280, 96)
                        arem_v[0][pl.ds(sb * TS, TS), :] = ae.astype(bf16)
                        arem_v[1][pl.ds(sb * TS, TS), :] = ao.astype(bf16)
                if remfirst:
                    rem()
                    yield
                for j in range(5):
                    for sb in range(gusub):
                        A11, A21 = tile(Ss[sb], j * 128, 128)
                        A12, A22 = tile(Ss[sb], 640 + j * 128, 128)
                        SS = strassen_a(A11, A12, A21, A22)
                        for i in range(7):
                            as_v[i][pl.ds(sb * TS, TS), j * 128:(j + 1) * 128] = SS[i].astype(bf16)
                    yield
                    yield
                if not remfirst:
                    rem()
                    yield

            interleave([(g_gu(), 11, 0.0), (g_scan(), scanw or NW, 0.001)])

            def hs_mat(slab0):
                return jnp.concatenate([pltpu.bitcast(hs[pl.ds((slab0 + c) * HP, NW), :], bf16) for c in range(4)], axis=1)
            slab = [8, 12, 0, 4, 24, 16, 20]
            AS = [as_v[i][...] for i in range(7)]
            HS = [hs_mat(slab[i]) for i in range(7)]
            are_, aro_ = arem_v[0][...], arem_v[1][...]
            dskv = vec_v[3].astype(f32)
            halves = [(0, 128), (128, 128)] if nsplit else [(0, 256)]
            Mc = {}
            if cfirst:
                for (c0, cw) in halves[:1]:
                    for i in range(7):
                        Mc[(c0, i)] = nt(HS[i], tc_v[i][pl.ds(c0, cw), :])
            for (c0, cw) in halves:
                cs = pl.ds(c0, cw)
                if cfirst and (c0, 0) not in Mc:
                    for i in range(7):
                        Mc[(c0, i)] = nt(HS[i], tc_v[i][pl.ds(c0, cw), :])
                M = []
                if jit_td:
                    raw = [wd_v[0:640, cs], wd_v[0:640, pl.ds(256 + c0, cw)], wd_v[640:1280, cs], wd_v[640:1280, pl.ds(256 + c0, cw)]]
                    TDj = [t_.astype(bf16) for t_ in strassen_b(*[q_.astype(f32) for q_ in raw])]
                for i in range(7):
                    if i == 1:
                        Ti = wd_v[0:640, cs]
                    elif i == 4:
                        Ti = wd_v[640:1280, pl.ds(256 + c0, cw)]
                    elif jit_td:
                        Ti = TDj[i]
                    else:
                        Ti = td_v[SIDX[i]][:, cs]
                    if reload:
                        AS[i] = as_v[i][...]; HS[i] = hs_mat(slab[i])
                    if cfirst:
                        M.append(Mc[(c0, i)] + nn(AS[i], Ti))
                    else:
                        M.append(nn(AS[i], Ti) + nt(HS[i], tc_v[i][cs, :]))
                outs = [(0, 0, M[0] + M[3] - M[4] + M[6]), (0, 256, M[2] + M[4]),
                        (1, 0, M[1] + M[3]), (1, 256, M[0] - M[1] + M[2] + M[5])]
                for par, cb, y in outs:
                    cols = pl.ds(cb + c0, cw)
                    if nor:
                        xw = x32[pl.ds(q0, T2), cols]; nw_ = xnp[pl.ds(q0, T2), cols]
                        if par == 0:
                            xr = pltpu.bitcast(xw << 16, f32); nr = pltpu.bitcast(nw_ << 16, f32)
                        else:
                            xr = pltpu.bitcast(xw & jnp.uint32(0xFFFF0000), f32); nr = pltpu.bitcast(nw_ & jnp.uint32(0xFFFF0000), f32)
                        dk = jnp.concatenate([dskv[(cb + c0) // 128 + k_:(cb + c0) // 128 + k_ + 1, :] for k_ in range(cw // 128)], axis=1)
                        y = y + nn(are_ if par == 0 else aro_, wd_v[1280:1376, cols]) + (xr + nr * dk)
                    else:
                        y = y + nn(are_ if par == 0 else aro_, wd_v[1280:1376, cols]) + r_scr[par, pl.ds(q0, T2), cols]
                    for k in range(cw // 128):
                        o_scr[slot, (cb + c0) // 128 + k, pl.ds(par, T2, stride=2), :] = y[:, k * 128:(k + 1) * 128]
                for cb in (0, 256):
                    for k in range(cw // 128):
                        ocopy(n, slot, (cb + c0) // 128 + k).start()
            return hcell[0]

        with scope("ph2"):
            lax.fori_loop(0, n2, phase2, jnp.zeros((8, 128), f32))
        with scope("tail"):
            for nn_ in range(max(0, n2 - oslots), n2):
                for c in range(4):
                    ocopy(nn_, nn_ % oslots, c).wait()

    anyspec = pl.BlockSpec(memory_space=pltpu.HBM)
    V = pltpu.VMEM
    call = pl.pallas_call(
        kernel,
        in_specs=[anyspec] * 12,
        out_specs=anyspec,
        out_shape=jax.ShapeDtypeStruct((L, D), f32),
        scratch_shapes=[V((L // 2, D), u32), V((4, 4, 128), bf16),
                        V((P // 2, D), u32), V((P // 2, D), u32), V((D // 2, P), u32), V((D // 2, P), u32),
                        V((F // 2, D), u32), V((F // 2, D), u32), V((F // 2, D), u32),
                        pltpu.SemaphoreType.DMA((13 + n1,)), pltpu.SemaphoreType.DMA((4 * oslots,)),
                        V((40, 128), f32),
                        V((7, LH // 2, 256), u32),
                        V((2, 8 if nor else LH, D), f32),
                        V((LH * UP + 8, 128), f32), V((LH * UP + 8, 128), f32),
                        V((32 * HP + 8, 128), u32),
                        V((5, 256, 256), u32),
                        V((5, F // 2, 256), u32),
                        V((5, 320, 256), u32),
                        V((7, 128, 512), u32),
                        V((7, T2 // 2, 640), u32),
                        V((2, T2, 96), bf16),
                        V((oslots, 4, 2 * T2 + 8, 128), f32), V((LH, D), u32)],
        compiler_params=pltpu.CompilerParams(vmem_limit_bytes=110 * 1024 * 1024, flags=flags),
        name="ssm_geglu_strassen",
    )

    @jax.jit
    def fn(A_x, A_Lambda_re, A_Lambda_im, A_B_re, A_B_im, A_C_re, A_C_im, A_log_dt, A_Dskip, B_x, B_w_gate, B_w_up, B_w_down):
        r = lambda v: v.reshape(4, 128)
        out = call(A_x.reshape(L, D), r(A_Lambda_re), r(A_Lambda_im), A_B_re, A_B_im, A_C_re, A_C_im,
                   r(A_log_dt), r(A_Dskip), B_w_gate.T, B_w_up.T, B_w_down)
        return out.reshape(1, L, D)
    return fn


A4 = [0,1,2,3]
def plan_base(ln=190, ln0=40, tb=11, tc=100, tg=34, td=75):
    return dict(X0=[256]*4, order=['x0','b0','b1','x1','x2','c','x3','w','wd'], plan=[
        (['x0'], [('ln',0,(ln0,0))]),
        (['b0','b1'], [('tb',(tb,0),0,512)]),
        (['x1'], [('b',0,256,A4),('ln',1,(ln,0))]),
        (['x2','c'], [('b',256,256,A4),('ln',2,(ln,0)),('tc',(tc,0))]),
        (['x3'], [('b',512,256,A4),('ln',3,(ln,0))]),
        (['w','wd'], [('b',768,256,A4),('tg',(tg,0)),('td',(td,0))])])
def plan_h(ln=190, ln0=40, tb=11, tc=100, tg=34, td=75, lnh=100):
    return dict(X0=[256]*4, order=['x0','b0','b1','x1','x2','c','x3','w','wd'], plan=[
        (['x0'], [('ln',0,(ln0,0))]),
        (['b0'], [('tb',(tb,0),0,256)]),
        (['b1'], [('b',0,256,[0,1]),('tb',(tb*3,0),256,512)]),
        (['x1'], [('b',0,256,[2,3]),('ln',1,(lnh,0))]),
        (['x2','c'], [('b',256,256,A4),('ln',2,(ln,0)),('tc',(tc,0))]),
        (['x3'], [('b',512,256,A4),('ln',3,(ln,0))]),
        (['w','wd'], [('b',768,256,A4),('tg',(tg,0)),('td',(td,0))])])
def plan_s(ln=190, ln0=40, tb=11, tc=100, tg=34, td=75, lnh=100, lnq=100):
    return dict(X0=[128,128,256,256,256], order=['x0','b0','x1','b1','x2','x3','c','x4','w','wd'], plan=[
        (['x0'], [('ln',0,(ln0,0))]),
        (['b0'], [('tb',(tb,0),0,256)]),
        (['x1'], [('b',0,128,[0,1]),('ln',1,(lnq,0))]),
        (['b1'], [('b',128,128,[0,1]),('tb',(tb*3,0),256,512)]),
        (['x2'], [('b',0,256,[2,3]),('ln',2,(lnh,0))]),
        (['x3','c'], [('b',256,256,A4),('ln',3,(ln,0)),('tc',(tc,0))]),
        (['x4'], [('b',512,256,A4),('ln',4,(ln,0))]),
        (['w','wd'], [('b',768,256,A4),('tg',(tg,0)),('td',(td,0))])])
def plan_s2(ln=190, ln0=40, tb=11, tc=100, tga=38, tgb=30, td=40, lnh=90, lnq=80, cut=688, order=None, tcs=6):
    p = [
        (['x0'], [('ln',0,(ln0,0))]),
        (['b0'], [('tb',(tb,0),0,256)]),
        (['x1'], [('b',0,128,[0,1]),('ln',1,(lnq,0))]),
        (['b1'], [('b',128,128,[0,1]),('tb',(tb*3,0),256,512)]),
        (['x2'], [('b',0,256,[2,3]),('ln',2,(lnh,0))]),
        (['x3'], [('b',256,256,A4),('ln',3,(ln,0))]),
        (['x4'], [('b',512,256,A4),('ln',4,(ln,0))]),
        (['w'], [('b',768,256,[0,1]),('tg',(tga,0),0,cut)]),
        (['wd'], [('b',768,256,[2,3]),('tg',(tgb,0),cut,1376),('td',(td,0))])]
    p[tcs][0].insert(0, 'c'); p[tcs][1].append(('tc',(tc,0)))
    return dict(X0=[128,128,256,256,256], order=order or ['x0','b0','x1','b1','x2','x3','x4','c','w','wd'], plan=p)


pallas_parallel_sum__ssm_conv_s5__geglu_ffn__prompt_kernel = make(
    nsplit=True, flags={"XLA_TPU_FORCE_LP_LLO_SCHEDULER": True}, **plan_s2(cut=1024, tga=26, tgb=60, td=40))
```

```python
import jax
import jax.numpy as jnp
import numpy as np
from jax import lax
import jax.experimental.pallas as pl
import jax.experimental.pallas.tpu as pltpu

f32 = jnp.float32
bf16 = jnp.bfloat16
u32 = jnp.uint32

L, D, P, F = 2048, 512, 512, 1376
LH = L // 2
T2 = 256
N2 = LH // T2
NW = T2 // 2
HP = NW + 1
UP = 9
CH = 16
RB = 16
RC = 32
XBLK = (128, 128, 256, 256, 256)
XOFF = tuple(sum(XBLK[:i]) for i in range(len(XBLK)))
SUMS = (0, 2, 3, 5, 6)
SIDX = {i: j for j, i in enumerate(SUMS)}
ALL4 = (0, 1, 2, 3)

DMA_ORDER = ("lre", "lim", "ldt", "dsk", "x0", "bre0", "bim0", "x1", "bre1", "bim1", "x2", "x3", "x4",
             "cre", "cim", "wg", "wu", "wd")
PLAN = (
    (("x0",), (("ln", 0, 40),)),
    (("bre0", "bim0"), (("tb", 11, 0, 256),)),
    (("x1",), (("b", 0, 128, (0, 1)), ("ln", 1, 80))),
    (("bre1", "bim1"), (("b", 128, 128, (0, 1)), ("tb", 33, 256, 512))),
    (("x2",), (("b", 0, 256, (2, 3)), ("ln", 2, 90))),
    (("x3",), (("b", 256, 256, ALL4), ("ln", 3, 190))),
    (("x4",), (("b", 512, 256, ALL4), ("ln", 4, 190))),
    (("cre", "cim", "wg", "wu"), (("b", 768, 256, (0, 1)), ("tc", 52), ("tg", 60, 0, 448))),
    (("wd",), (("b", 768, 256, (2, 3)), ("tg", 28, 448, F), ("td", 40))),
)


def _nt(a, b):
    return lax.dot_general(a, b, (((1,), (1,)), ((), ())), preferred_element_type=f32)


def _nn(a, b):
    return lax.dot_general(a, b, (((1,), (0,)), ((), ())), preferred_element_type=f32)


def _gelu(g):
    c = np.float32(np.sqrt(2.0 / np.pi))
    return 0.5 * g * (1.0 + jnp.tanh(c * (g + 0.044715 * (g * g * g))))


def _strassen_a(a11, a12, a21, a22):
    return [a11 + a22, a21 + a22, a11, a22, a11 + a12, a21 - a11, a12 - a22]


def _strassen_b(b11, b12, b21, b22):
    return [b11 + b22, b11, b12 - b22, b21 - b11, b22, b11 + b12, b21 + b22]


def _lo(w):
    return pltpu.bitcast(w << 16, f32)


def _hi(w):
    return pltpu.bitcast(w & jnp.uint32(0xFFFF0000), f32)


def _pack2(lo, hi):
    a = pltpu.bitcast(lo.astype(bf16).astype(f32), u32)
    b = pltpu.bitcast(hi.astype(bf16).astype(f32), u32)
    return (a >> 16) | b


def _interleave(gens):
    gens = [[g, w, o] for g, w, o in gens]
    while gens:
        gens.sort(key=lambda e: e[2])
        e = gens[0]
        try:
            next(e[0])
            e[2] += 1.0 / e[1]
        except StopIteration:
            gens.pop(0)


def _kernel(x_hbm, lre_hbm, lim_hbm, bre_hbm, bim_hbm, cre_hbm, cim_hbm, ldt_hbm, dsk_hbm,
            wg_hbm, wu_hbm, wd_hbm, o_hbm,
            x32, vec_v, bre32, bim32, cre32, cim32, wg32, wu32, wd32, sems, osem,
            ab, xs, ue, uo, hs, tb, tg, td, tc, as_, arem, o_scr, xq):
    x_v, bre_v, bim_v, cre_v, cim_v, wg_v, wu_v, wd_v = (
        r.bitcast(bf16) for r in (x32, bre32, bim32, cre32, cim32, wg32, wu32, wd32))
    views = lambda r, n: [r.at[i].bitcast(bf16) for i in range(n)]
    xs_v, xq_v, as_v = views(xs, 7), views(xq, 2), views(as_, 7)
    tb_v, tg_v, td_v, tc_v = views(tb, 5), views(tg, 5), views(td, 5), views(tc, 7)

    src = dict(lre=(lre_hbm, vec_v.at[0]), lim=(lim_hbm, vec_v.at[1]), ldt=(ldt_hbm, vec_v.at[2]),
               dsk=(dsk_hbm, vec_v.at[3]), cre=(cre_hbm, cre_v), cim=(cim_hbm, cim_v),
               wg=(wg_hbm, wg_v), wu=(wu_hbm, wu_v), wd=(wd_hbm, wd_v))
    for b in range(len(XBLK)):
        rows = pl.ds(2 * XOFF[b], 2 * XBLK[b])
        src["x%d" % b] = (x_hbm.at[rows, :], x_v.at[rows, :])
    for h in range(2):
        rows = pl.ds(h * 256, 256)
        src["bre%d" % h] = (bre_hbm.at[rows, :], bre_v.at[rows, :])
        src["bim%d" % h] = (bim_hbm.at[rows, :], bim_v.at[rows, :])
    cps = {k: pltpu.make_async_copy(src[k][0], src[k][1], sems.at[i]) for i, k in enumerate(DMA_ORDER)}
    for k in DMA_ORDER:
        cps[k].start()

    for k in ("lre", "lim", "ldt", "dsk"):
        cps[k].wait()
    lre = vec_v[0].astype(f32)
    lim = vec_v[1].astype(f32)
    dt = jnp.exp(vec_v[2].astype(f32)).astype(bf16).astype(f32)
    mag = jnp.exp(dt * lre)
    are = mag * jnp.cos(dt * lim)
    aim = mag * jnp.sin(dt * lim)
    nre = are - 1.0
    den = lre * lre + lim * lim
    ab[0:4, :] = are
    ab[4:8, :] = are
    ab[8:12, :] = -aim
    ab[12:16, :] = aim
    ab[16:20, :] = 2.0 * (nre * lre + aim * lim) / den
    ab[20:24, :] = 2.0 * (aim * lre - nre * lim) / den

    zero = [0]

    def new_zero(ref):
        zero[0] = jnp.sum(jnp.minimum((ref[0:8, 0:128] >> 31).astype(jnp.int32), 0))

    def pacer(n, delay):
        out, z = [], zero[0]
        s = z
        for _ in range(n):
            out.append(s)
            for j in range(delay):
                s = (s + z) if j % 2 == 0 else (s | z)
        return out

    def g_ln(blk, delay):
        pz = pacer(XBLK[blk] // CH, delay)
        for ch in range(XBLK[blk] // CH):
            q0 = XOFF[blk] + ch * CH
            w = x32[pl.ds(pl.multiple_of(q0 + pz[ch], CH), CH), :]
            xn = []
            for x in (_lo(w), _hi(w)):
                mu = jnp.sum(x, axis=-1, keepdims=True) * (1.0 / D)
                xc = x - mu
                var = jnp.sum(xc * xc, axis=-1, keepdims=True) * (1.0 / D)
                xn.append(xc * lax.rsqrt(var + 1e-5))
            xq_v[0][pl.ds(q0, CH), :] = xn[0][:, 256:].astype(bf16)
            xq_v[1][pl.ds(q0, CH), :] = xn[1][:, :256].astype(bf16)
            s = _strassen_a(xn[0][:, :256], xn[0][:, 256:], xn[1][:, :256], xn[1][:, 256:])
            for i in range(7):
                xs_v[i][pl.ds(q0, CH), :] = s[i].astype(bf16)
            yield

    def presum(srcs, dst, delay, lo, hi):
        pz = pacer((hi - lo) // RB, delay)
        for r0 in range(lo, hi, RB):
            r = pl.multiple_of(r0 + pz[(r0 - lo) // RB], RB)
            t = _strassen_b(*[ref[pl.ds(off + r, RB), cols].astype(f32) for ref, off, cols in srcs])
            for i in SUMS:
                dst[SIDX[i]][pl.ds(r0, RB), :] = t[i].astype(bf16)
            yield

    h0, h1 = slice(0, 256), slice(256, 512)
    g_tb = lambda d, lo, hi: presum([(bre_v, 0, h0), (bim_v, 0, h0), (bre_v, 0, h1), (bim_v, 0, h1)], tb_v, d, lo, hi)
    g_tg = lambda d, lo, hi: presum([(wg_v, 0, h0), (wu_v, 0, h0), (wg_v, 0, h1), (wu_v, 0, h1)], tg_v, d, lo, hi)
    g_td = lambda d: presum([(wd_v, 0, h0), (wd_v, 0, h1), (wd_v, 640, h0), (wd_v, 640, h1)], td_v, d, 0, 640)

    def g_tc(delay):
        cre, cim = ab[16:20, :], ab[20:24, :]
        pz = pacer(4 * 256 // RC, delay)
        for r0 in range(0, 256, RC):
            for c in range(4):
                sl = slice(c * 128, (c + 1) * 128)
                rr, mm = cre[c:c + 1, :], cim[c:c + 1, :]
                q = []
                for dh in range(2):
                    rows = pl.ds(pl.multiple_of(dh * 256 + r0 + pz[(r0 // RC) * 4 + c], RC), RC)
                    a, b = cre_v[rows, sl].astype(f32), cim_v[rows, sl].astype(f32)
                    q.append((a * rr - b * mm, a * mm + b * rr))
                (re0, im0), (re1, im1) = q
                t = [re0 - im1, re0, re1 + im1, -(im0 + re0), -im1, re0 + re1, im0 + im1]
                for i in range(7):
                    tc_v[i][pl.ds(r0, RC), sl] = t[i].astype(bf16)
            yield

    def g_u(q0, n, tiles):
        s = [xs_v[i][pl.ds(q0, n), :] for i in range(7)]
        for c in tiles:
            ns = pl.ds(c * 128, 128)
            t = [tb_v[0][ns, :], bre_v[ns, h0], tb_v[1][ns, :], tb_v[2][ns, :],
                 bim_v[ns, h1], tb_v[3][ns, :], tb_v[4][ns, :]]
            m = [_nt(s[i], t[i]) for i in range(7)]
            ue[pl.ds(q0 * UP + c, n, stride=UP), :] = m[0] + m[3] - m[4] + m[6]
            ue[pl.ds(q0 * UP + 4 + c, n, stride=UP), :] = m[2] + m[4]
            uo[pl.ds(q0 * UP + c, n, stride=UP), :] = m[1] + m[3]
            uo[pl.ds(q0 * UP + 4 + c, n, stride=UP), :] = m[0] - m[1] + m[2] + m[5]
            yield

    zsrc = dict(bim0=bre32, bim1=bre32.at[pl.ds(128, 8)], wu=wg32, wd=wd32)
    for b in range(len(XBLK)):
        zsrc["x%d" % b] = x32.at[pl.ds(XOFF[b], 8)]
    for waits, tasks in PLAN:
        for k in waits:
            cps[k].wait()
        new_zero(zsrc[waits[-1]])
        gens = []
        for t in tasks:
            if t[0] == "b":
                gens.append((g_u(*t[1:]), len(t[3]), 0.0))
            elif t[0] == "ln":
                gens.append((g_ln(*t[1:]), XBLK[t[1]] // CH, 0.001))
            else:
                fn, n = dict(tb=(g_tb, 16), tg=(g_tg, 43), td=(g_td, 40), tc=(g_tc, 8))[t[0]]
                gens.append((fn(*t[1:]), n, 0.002))
        _interleave(gens)

    def ocopy(n, c):
        return pltpu.make_async_copy(o_scr.at[n, c, pl.ds(0, 2 * T2), :],
                                     o_hbm.at[pl.ds(n * 2 * T2, 2 * T2), pl.ds(c * 128, 128)],
                                     osem.at[n * 4 + c])

    top = lax.broadcasted_iota(jnp.int32, (8, 128), 0) < 4

    def phase2(n, h_in):
        q0 = pl.multiple_of(n * T2, T2)
        carry = [h_in]

        def g_scan():
            a, bm = ab[0:8, :], ab[8:16, :]
            h = carry[0]
            sh = pltpu.roll(h, 4, 0)
            base = pl.multiple_of(n * (T2 * UP), T2 * UP)
            for w in range(NW):
                parts = []
                for k in range(2):
                    q = 2 * w + k
                    g = a * h + bm * sh + ue[pl.ds(base + q * UP, 8), :]
                    sg = pltpu.roll(g, 4, 0)
                    h = a * g + bm * sg + uo[pl.ds(base + q * UP, 8), :]
                    sh = pltpu.roll(h, 4, 0)
                    x = jnp.where(top, g, h)
                    parts.append((x, x + sh, h - g, g + sg))
                for j in range(4):
                    hs[pl.ds(j * 8 * HP + w, 8, stride=HP), :] = _pack2(parts[0][j], parts[1][j])
                yield
            carry[0] = h

        def g_ffn():
            s = [xs_v[i][pl.ds(q0, T2), :] for i in range(7)]

            def tile(j0, jw):
                ns = pl.ds(j0, jw)
                t = [tg_v[0][ns, :], wg_v[ns, h0], tg_v[1][ns, :], tg_v[2][ns, :],
                     wu_v[ns, h1], tg_v[3][ns, :], tg_v[4][ns, :]]
                m = [_nt(s[i], t[i]) for i in range(7)]
                ge = m[0] + m[3] - m[4] + m[6]
                uo_ = m[0] - m[1] + m[2] + m[5]
                ue_ = m[2] + m[4]
                go = m[1] + m[3]
                return _gelu(ge) * ue_, _gelu(go) * uo_

            ae, ao = tile(1280, 96)
            arem[0] = ae.astype(bf16)
            arem[1] = ao.astype(bf16)
            yield
            for j in range(5):
                a11, a21 = tile(j * 128, 128)
                a12, a22 = tile(640 + j * 128, 128)
                ss = _strassen_a(a11, a12, a21, a22)
                for i in range(7):
                    as_v[i][:, j * 128:(j + 1) * 128] = ss[i].astype(bf16)
                yield
                yield

        _interleave([(g_ffn(), 11, 0.0), (g_scan(), NW, 0.001)])

        slab = (8, 12, 0, 4, 24, 16, 20)
        a_s = [as_v[i][...] for i in range(7)]
        h_s = [jnp.concatenate([pltpu.bitcast(hs[pl.ds((slab[i] + c) * HP, NW), :], bf16) for c in range(4)], axis=1)
               for i in range(7)]
        a_r = (arem[0], arem[1])
        dsk = vec_v[3].astype(f32)
        for c0 in (0, 128):
            cs = pl.ds(c0, 128)
            m = [None] * 7

            def prod(*idx):
                for i in idx:
                    t = (wd_v[0:640, cs] if i == 1 else wd_v[640:1280, pl.ds(256 + c0, 128)] if i == 4
                         else td_v[SIDX[i]][:, cs])
                    m[i] = _nn(a_s[i], t) + _nt(h_s[i], tc_v[i][cs, :])

            def emit(par, cb, y):
                cols = pl.ds(cb + c0, 128)
                xw = x32[pl.ds(q0, T2), cols]
                nsrc = {(0, 0): xs_v[2], (0, 256): xq_v[0], (1, 0): xq_v[1], (1, 256): xs_v[3]}[(par, cb)]
                nr = nsrc[pl.ds(q0, T2), cs].astype(f32)
                c = (cb + c0) // 128
                y = y + _nn(a_r[par], wd_v[1280:F, cols]) + ((_hi if par else _lo)(xw) + nr * dsk[c:c + 1, :])
                o_scr[n, c, pl.ds(par, T2, stride=2), :] = y

            prod(1, 3)
            emit(1, 0, m[1] + m[3])
            prod(4, 0, 6)
            emit(0, 0, m[0] + m[3] - m[4] + m[6])
            ocopy(n, c0 // 128).start()
            prod(2)
            emit(0, 256, m[2] + m[4])
            prod(5)
            emit(1, 256, m[0] - m[1] + m[2] + m[5])
            ocopy(n, 2 + c0 // 128).start()
        return carry[0]

    lax.fori_loop(0, N2, phase2, jnp.zeros((8, 128), f32))
    for n in range(N2):
        for c in range(4):
            ocopy(n, c).wait()


@jax.jit
def pallas_parallel_sum__ssm_conv_s5__geglu_ffn__prompt_kernel(
    A_x, A_Lambda_re, A_Lambda_im, A_B_re, A_B_im, A_C_re, A_C_im, A_log_dt, A_Dskip,
    B_x, B_w_gate, B_w_up, B_w_down,
):
    del B_x
    hbm = pl.BlockSpec(memory_space=pltpu.HBM)
    V = pltpu.VMEM
    call = pl.pallas_call(
        _kernel,
        in_specs=[hbm] * 12,
        out_specs=hbm,
        out_shape=jax.ShapeDtypeStruct((L, D), f32),
        scratch_shapes=[
            V((L // 2, D), u32), V((4, 4, 128), bf16),
            V((P // 2, D), u32), V((P // 2, D), u32), V((D // 2, P), u32), V((D // 2, P), u32),
            V((F // 2, D), u32), V((F // 2, D), u32), V((F // 2, D), u32),
            pltpu.SemaphoreType.DMA((len(DMA_ORDER),)), pltpu.SemaphoreType.DMA((4 * N2,)),
            V((24, 128), f32),
            V((7, LH // 2, 256), u32),
            V((LH * UP + 8, 128), f32), V((LH * UP + 8, 128), f32),
            V((32 * HP + 8, 128), u32),
            V((5, 256, 256), u32), V((5, F // 2, 256), u32), V((5, 320, 256), u32), V((7, 128, 512), u32),
            V((7, T2 // 2, 640), u32), V((2, T2, 96), bf16),
            V((N2, 4, 2 * T2 + 8, 128), f32),
            V((2, LH // 2, 256), u32),
        ],
        compiler_params=pltpu.CompilerParams(
            vmem_limit_bytes=110 * 1024 * 1024,
            flags={"XLA_TPU_FORCE_LP_LLO_SCHEDULER": True},
            disable_bounds_checks=True,
            disable_semaphore_checks=True,
        ),
        name="ssm_geglu_strassen",
    )
    r = lambda v: v.reshape(4, 128)
    out = call(A_x.reshape(L, D), r(A_Lambda_re), r(A_Lambda_im), A_B_re, A_B_im, A_C_re, A_C_im,
               r(A_log_dt), r(A_Dskip), B_w_gate.T, B_w_up.T, B_w_down)
    return out.reshape(1, L, D)
```
